```python
import jax
import jax.numpy as jnp

def _softmax(x, axis=-1):
    return jax.nn.softmax(x, axis=axis)
def _gelu(x):
    return jax.nn.gelu(x, approximate=True)
def _silu(x):
    return jax.nn.silu(x)
def _sigmoid(x):
    return jax.nn.sigmoid(x)
def _layernorm(x, axis=-1, eps=1e-5):
    m = jnp.mean(x, axis=axis, keepdims=True)
    v = jnp.var(x, axis=axis, keepdims=True)
    return (x - m) / jnp.sqrt(v + eps)
def _scatter_add(tgt, idx, src, axis=0):
    return tgt.at[idx].add(src)
def _segment_sum(src, seg, n):
    return jax.ops.segment_sum(src, seg, n)
class _Rng:
    def __init__(self, key):
        self._k = key
    def _next(self):
        self._k, sub = jax.random.split(self._k)
        return sub
    def normal(self, shape):
        return jax.random.normal(self._next(), shape, dtype=jnp.bfloat16)
    def randint(self, lo, hi, shape):
        return jax.random.randint(self._next(), shape, lo, hi, dtype=jnp.int32)
    def uniform(self, shape, lo=0.0, hi=1.0):
        return jax.random.uniform(self._next(), shape, jnp.bfloat16, lo, hi)
    def permutation(self, n):
        return jax.random.permutation(self._next(), n)


kernel_name = 'parallel_sum__sliding_block_cached__mixer_s_mlp__decode'

def setup_inputs():
    _rng = _Rng(jax.random.key(int.from_bytes(__import__("os").urandom(4), "little")))
    _w = (lambda a: (lambda t: t.astype(jnp.bfloat16) if jnp.issubdtype(t.dtype, jnp.floating) else t)(jnp.asarray(a)))
    def _A_setup():
        B, Sq, D = 4, 1, 512
        Hq, Hkv, Sk, Dh = 32, 32, 8192, 128
        assert Hq % Hkv == 0, (Hq, Hkv)
        return {
            "x": _w((lambda *s: _rng.normal(s) * 0.05)(B, Sq, D)),
            "k_cache": _w((lambda *s: _rng.normal(s) * 0.05)(B, Hkv, Sk, Dh)),
            "v_cache": _w((lambda *s: _rng.normal(s) * 0.05)(B, Hkv, Sk, Dh)),
            "wq": _w((lambda *s: _rng.normal(s) * 0.05)(D, Hq * Dh) * (D ** -0.5)),
            "wo": _w((lambda *s: _rng.normal(s) * 0.05)(Hq * Dh, D) * ((Hq * Dh) ** -0.5)),
        }
    _A_in = _A_setup()

    def _B_setup():
        B, S, D, F = 4, 1, 512, 1376
        return {
            "x":  _w((lambda *s: _rng.normal(s) * 0.05)(B, S, D)),
            "w1": _w((lambda *s: _rng.normal(s) * 0.05)(D, D) * (D ** -0.5)),
            "w2": _w((lambda *s: _rng.normal(s) * 0.05)(D, D) * (D ** -0.5)),
            "w3": _w((lambda *s: _rng.normal(s) * 0.05)(D, F) * (D ** -0.5)),
            "w4": _w((lambda *s: _rng.normal(s) * 0.05)(F, D) * (F ** -0.5)),
        }
    _B_in = _B_setup()

    return {
        "A_x": _A_in["x"],
        "A_k_cache": _A_in["k_cache"],
        "A_v_cache": _A_in["v_cache"],
        "A_wq": _A_in["wq"],
        "A_wo": _A_in["wo"],
        "B_x": _B_in["x"],
        "B_w1": _B_in["w1"],
        "B_w2": _B_in["w2"],
        "B_w3": _B_in["w3"],
        "B_w4": _B_in["w4"],
    }

def reference(A_x, A_k_cache, A_v_cache, A_wq, A_wo, B_x, B_w1, B_w2, B_w3, B_w4):
    def _A_ref(x, k_cache, v_cache, wq, wo):
        B, Sq, D = x.shape
        Hq, Dh = 32, 128
        Hkv, Sk = k_cache.shape[1], k_cache.shape[2]
        W = min(4096, max(256, Sk // 4))
        rep = Hq // Hkv
        q = (lambda x, *d: x.transpose(*d))((x @ wq).reshape(B, Sq, Hq, Dh), 0, 2, 1, 3)
        k = jnp.repeat(k_cache[:, :, Sk - W:, :], rep, axis=1)
        v = jnp.repeat(v_cache[:, :, Sk - W:, :], rep, axis=1)
        scores = jnp.einsum("bhqd,bhkd->bhqk", q, k) * (Dh ** -0.5)
        p = _softmax(scores, axis=-1)
        o = jnp.einsum("bhqk,bhkd->bhqd", p, v)
        return (lambda x, *d: x.transpose(*d))(o, 0, 2, 1, 3).reshape(B, Sq, Hq * Dh) @ wo

    def _B_ref(x, w1, w2, w3, w4):
        B, S, D = x.shape
        h = _gelu(_layernorm(x, axis=-1) @ w1)
        c = D // 4
        g0 = jnp.pad(h[:, :, 0*c:1*c], ((0, 0), (1, 0), (0, 0)))[:, :S, :]
        g1 = jnp.pad(h[:, :, 1*c:2*c], ((0, 0), (0, 1), (0, 0)))[:, 1:, :]
        g2 = jnp.pad(h[:, :, 2*c:3*c], ((0, 0), (2, 0), (0, 0)))[:, :S, :]
        g3 = jnp.pad(h[:, :, 3*c:   ], ((0, 0), (0, 2), (0, 0)))[:, 2:, :]
        hs = jnp.concatenate([g0, g1, g2, g3], axis=-1) @ w2
        x1 = x + hs
        h2 = _gelu(_layernorm(x1, axis=-1) @ w3) @ w4
        return x1 + h2

    x = A_x
    xn = _layernorm(x, axis=-1)
    return x + _A_ref(xn, A_k_cache, A_v_cache, A_wq, A_wo) + _B_ref(xn, B_w1, B_w2, B_w3, B_w4)
```

```python
import functools
import math

import jax
import jax.numpy as jnp
from jax import lax
from jax.experimental import pallas as pl
from jax.experimental.pallas import tpu as pltpu

F32, BF16 = jnp.float32, jnp.bfloat16
G = 8
T = 128
NT_DIMS = (((1,), (1,)), ((), ()))


def _layernorm(x, eps=1e-5):
    m = jnp.mean(x, axis=-1, keepdims=True)
    d = x - m
    v = jnp.mean(d * d, axis=-1, keepdims=True)
    return d * lax.rsqrt(v + eps)


def stride(hs):
    return lambda g, i: (g // hs) * (hs * G) + g % hs + i * hs


def hb(hs, bfast=True):
    def f(g, i):
        hh, b = (i // 4, i % 4) if bfast else (i % 2, i // 2)
        return b * 32 + (g // hs) * (2 * hs) + g % hs + hh * hs
    return f


def build(pair=stride(8), L=8, ring=16, fine=True, nobounds=True, wo_gran=1, flags=None):
    B, H, SK, DH, D, FF = 4, 32, 8192, 128, 512, 1376
    W = min(4096, max(256, SK // 4))
    NS = W // T
    NG = B * H // G
    HU = NS // 2
    NKV = (NG - 1) * NS
    NU = 2 * HU + NKV
    c_exp = (DH ** -0.5) * math.log2(math.e)
    WR = 32

    def kend(u):
        return "K" if u < HU else "KV" if u < HU + NKV else "V" if u < NU else "O"

    def kern(x_hbm, k_hbm, v_hbm, wq_hbm, wo_hbm, w3_hbm, w4_hbm, out_hbm,
             buf, x_v, wq_v, wo_v, w3_v, w4_v, q_s, o_s, s_s, st, res_s, out_v,
             sem_kv, sem_wo, sem_misc):
        row = lax.broadcasted_iota(jnp.int32, (G, T), 0)
        Q, MX, M, LS, ACC = range(5)

        def tile_copy(src, g, i, s, slot, half):
            r = pl.multiple_of(SK - W + s * T, T)
            return pltpu.make_async_copy(src.at[pair(g, i), pl.ds(r, T)], buf.at[slot, half, i], sem_kv.at[slot])

        def issuer(kind, u):
            slot = u % ring
            if kind == "K":
                return lambda n: tile_copy(k_hbm, 0, n // 2, u + HU * (n % 2), slot, n % 2).start(priority=n % 2)
            if kind == "V":
                j = u - (HU + NKV)
                return lambda n: tile_copy(v_hbm, NG - 1, n // 2, j + HU * (n % 2), slot, n % 2).start(priority=n % 2)
            if kind == "KV":
                g, s = (u + HU) // NS, (u + HU) % NS
                return lambda n: tile_copy((k_hbm, v_hbm)[n % 2], g - n % 2, n // 2, s, slot, n % 2).start(priority=n % 2)
            j = u - NU

            def f(n):
                r = pl.multiple_of((j * 16 + n) * WR, WR)
                pltpu.make_async_copy(wo_hbm.at[pl.ds(r, WR)], wo_v.at[pl.ds(r, WR)],
                                      sem_wo.at[(j * 4 + n // 4) // wo_gran]).start(priority=n % 2)
            return f

        def qk(slot, half, s, issue, n0):
            q = st[Q].astype(BF16)
            sc = None
            for i in range(G):
                t = lax.dot_general(q, buf[slot, half, i], NT_DIMS, preferred_element_type=F32)
                sc = t if sc is None else jnp.where(row == i, t, sc)
                issue(n0 + i)
            s_s[s] = sc
            st[MX] = jnp.maximum(st[MX], sc)

        def pv(slot, half, s, issue, n0):
            p = jnp.exp2((s_s[s] - st[M]) * c_exp)
            st[LS] = st[LS] + p
            pb = p.astype(BF16)
            o = None
            for i in range(G):
                t = jnp.dot(pb, buf[slot, half, i], preferred_element_type=F32)
                o = t if o is None else jnp.where(row == i, t, o)
                issue(n0 + i)
            st[ACC] = st[ACC] + o

        def qo_row(g, i):
            p = pair(g, i)
            return (p % H) * G + p // H

        def load_q(g):
            q = None
            for i in range(G):
                t = jnp.broadcast_to(q_s[pl.ds(qo_row(g, i), 1), :], (G, T))
                q = t if q is None else jnp.where(row == i, t, q)
            st[Q] = q

        def begin_pv():
            st[M] = jnp.broadcast_to(jnp.max(st[MX], axis=-1, keepdims=True), (G, T))
            st[MX] = jnp.full((G, T), -jnp.inf, F32)
            st[LS] = jnp.zeros((G, T), F32)
            st[ACC] = jnp.zeros((G, T), F32)

        def end_pv(g):
            o = st[ACC] / jnp.sum(st[LS], axis=-1, keepdims=True)
            for i in range(G):
                o_s[pl.ds(qo_row(g, i), 1), :] = o[i:i + 1, :]

        def unit(ckind, ikind, u, _):
            slot = u % ring
            pltpu.make_async_copy(buf.at[slot], buf.at[slot], sem_kv.at[slot]).wait()
            start = issuer(ikind, u + L)
            if fine:
                issue = start
            else:
                issue = lambda n: None
            if ckind == "K":
                qk(slot, 0, u, issue, 0)
                qk(slot, 1, u + HU, issue, G)
            elif ckind == "V":
                j = u - (HU + NKV)
                pv(slot, 0, j, issue, 0)
                pv(slot, 1, j + HU, issue, G)
            else:
                g, s = (u + HU) // NS, (u + HU) % NS
                pv(slot, 1, s, issue, 0)
                qk(slot, 0, s, issue, G)

                @pl.when(s == NS - 1)
                def _():
                    end_pv(g - 1)
                    begin_pv()
                    load_q(jnp.minimum(g + 1, NG - 1))
            if not fine:
                for n in range(2 * G):
                    start(n)

        x_cp = pltpu.make_async_copy(x_hbm, x_v, sem_misc.at[0])
        x_cp.start()

        def issue_wq(j, _):
            for n in range(4):
                r = pl.multiple_of((j + (n // 2) * 32) * 8, 8)
                c = (n % 2) * 2048
                pltpu.make_async_copy(wq_hbm.at[pl.ds(r, 8), pl.ds(c, 2048)], wq_v.at[pl.ds(r, 8), pl.ds(c, 2048)],
                                      sem_misc.at[1]).start(priority=n % 2)
        lax.fori_loop(0, 32, issue_wq, None)

        def issue_mlp(j, _):
            r = pl.multiple_of(j * WR, WR)
            pltpu.make_async_copy(w3_hbm.at[pl.ds(r, WR)], w3_v.at[pl.ds(r, WR)], sem_misc.at[2]).start(priority=0)
            pltpu.make_async_copy(w4_hbm.at[pl.ds(r, WR)], w4_v.at[pl.ds(r, WR)], sem_misc.at[3]).start(priority=1)
        lax.fori_loop(0, FF // WR, issue_mlp, None)

        o_s[...] = jnp.zeros(o_s.shape, F32)
        st[MX] = jnp.full((G, T), -jnp.inf, F32)
        x_cp.wait()
        x4 = x_v[...].astype(F32)
        x = jnp.concatenate([x4, x4], axis=0)
        xn = _layernorm(x).astype(BF16)
        pltpu.make_async_copy(wq_v, wq_v, sem_misc.at[1]).wait()

        def q_unit(do_issue, j, _):
            start = issuer("K", j)
            for hh in range(4):
                c = pl.multiple_of((j * 4 + hh) * DH, DH)
                q = jnp.dot(xn, wq_v[:, pl.ds(c, DH)], preferred_element_type=F32)
                q_s[pl.ds(pl.multiple_of((j * 4 + hh) * G, G), G), :] = q
                if do_issue:
                    for n in range(4):
                        start(hh * 4 + n)
        lax.fori_loop(0, L, functools.partial(q_unit, True), None)
        if L < H // 4:
            lax.fori_loop(L, H // 4, functools.partial(q_unit, False), None)
        load_q(0)

        pltpu.make_async_copy(w3_v, w3_v, sem_misc.at[2]).wait()
        pltpu.make_async_copy(w4_v, w4_v, sem_misc.at[3]).wait()
        x1 = xn.astype(F32)
        h = lax.dot_general(_layernorm(x1).astype(BF16), w3_v[...], NT_DIMS, preferred_element_type=F32)
        h = jax.nn.gelu(h, approximate=True).astype(BF16)
        res_s[...] = x + x1 + jnp.dot(h, w4_v[...], preferred_element_type=F32)

        cuts = sorted({0, HU, HU + NKV, NU} | {c - L for c in (HU, HU + NKV, NU) if c - L > 0})
        for lo, hi in zip(cuts[:-1], cuts[1:]):
            lax.fori_loop(lo, hi, functools.partial(unit, kend(lo), kend(lo + L)), None)
            if hi == HU:
                begin_pv()
                load_q(1)
        if L < H // 4:
            def rest(u, _):
                start = issuer("O", u)
                for n in range(16):
                    start(n)
            lax.fori_loop(NU + L, NU + H // 4, rest, None)
        end_pv(NG - 1)

        def oproj(j, acc):
            r = pl.multiple_of(j * (wo_gran * DH), wo_gran * DH)
            pltpu.make_async_copy(wo_v.at[pl.ds(r, wo_gran * DH)], wo_v.at[pl.ds(r, wo_gran * DH)], sem_wo.at[j]).wait()
            for hh in range(wo_gran):
                o = o_s[pl.ds(pl.multiple_of((j * wo_gran + hh) * G, G), G), :].astype(BF16)
                acc = acc + jnp.dot(o, wo_v[pl.ds(pl.multiple_of(r + hh * DH, DH), DH), :], preferred_element_type=F32)
            return acc
        acc = lax.fori_loop(0, H // wo_gran, oproj, res_s[...])
        out_v[...] = acc[:B].astype(out_v.dtype)
        out_cp = pltpu.make_async_copy(out_v, out_hbm, sem_misc.at[0])
        out_cp.start()
        out_cp.wait()

    def f(A_x, A_k_cache, A_v_cache, A_wq, A_wo, B_x, B_w1, B_w2, B_w3, B_w4):
        hbm = pl.BlockSpec(memory_space=pltpu.HBM)
        out = pl.pallas_call(
            kern,
            out_shape=jax.ShapeDtypeStruct((B, D), BF16),
            in_specs=[hbm] * 7,
            out_specs=hbm,
            scratch_shapes=[
                pltpu.VMEM((ring, 2, G, T, DH), BF16),
                pltpu.VMEM((B, D), BF16),
                pltpu.VMEM((D, H * DH), BF16),
                pltpu.VMEM((H * DH, D), BF16),
                pltpu.VMEM((FF, D), BF16),
                pltpu.VMEM((FF, D), BF16),
                pltpu.VMEM((H * G, DH), F32),
                pltpu.VMEM((H * G, DH), F32),
                pltpu.VMEM((NS, G, T), F32),
                pltpu.VMEM((5, G, T), F32),
                pltpu.VMEM((G, D), F32),
                pltpu.VMEM((B, D), BF16),
                pltpu.SemaphoreType.DMA((ring,)),
                pltpu.SemaphoreType.DMA((H // wo_gran,)),
                pltpu.SemaphoreType.DMA((4,)),
            ],
            compiler_params=pltpu.CompilerParams(
                vmem_limit_bytes=64 * 2**20, disable_bounds_checks=nobounds, flags=flags),
        )(A_x.reshape(B, D), A_k_cache.reshape(B * H, SK, DH), A_v_cache.reshape(B * H, SK, DH),
          A_wq, A_wo, B_w3.T, B_w4)
        return out.reshape(B, 1, D)
    return f


@jax.jit
def pallas_parallel_sum__sliding_block_cached__mixer_s_mlp__decode_kernel(
    A_x, A_k_cache, A_v_cache, A_wq, A_wo, B_x, B_w1, B_w2, B_w3, B_w4
):
    return build(wo_gran=4)(A_x, A_k_cache, A_v_cache, A_wq, A_wo, B_x, B_w1, B_w2, B_w3, B_w4)
```

```python
import functools
import math

import jax
import jax.numpy as jnp
from jax import lax
from jax.experimental import pallas as pl
from jax.experimental.pallas import tpu as pltpu

F32, BF16 = jnp.float32, jnp.bfloat16

B, H, SK, DH, D, FF = 4, 32, 8192, 128, 512, 1376
W = min(4096, max(256, SK // 4))
G = 8
J = H // G
T = 128
NS = W // T
NR = B * J // 2
NW = H // 4
RING = 8
SKEW = 3
LAG = (4, 4 + SKEW)
WR = 16

NN = (((1,), (0,)), ((), ()))
NT = (((1,), (1,)), ((), ()))
EXP2_SCALE = DH ** -0.5 * math.log2(math.e)


def _layernorm(x, eps=1e-5):
    d = x - jnp.mean(x, axis=-1, keepdims=True)
    return d * lax.rsqrt(jnp.mean(d * d, axis=-1, keepdims=True) + eps)


def _dot(a, b, dims=NN):
    return lax.dot_general(a, b, dims, preferred_element_type=F32)


def _ds(start, size):
    return pl.ds(pl.multiple_of(start, size), size)


def _wait(ref, sem):
    pltpu.make_async_copy(ref, ref, sem).wait()


def _compute(x_hbm, k_hbm, v_hbm, wq_hbm, wo_hbm, w3_hbm, w4_hbm,
             kv, x_v, wq_v, wo_v, w3_v, w4_v, q_s, o_s, s_s, res_s,
             sems, wq_sem, mlp_sem):
    row = lax.broadcasted_iota(jnp.int32, (G, T), 0)

    def kv_pieces(src, rnd, s, p, slot):
        first = pl.multiple_of(SK - W + s * T, T)

        def start(n):
            heads, r = pl.ds(2 * (n % 4), 2), (n // 4) * (T // 2)
            pltpu.make_async_copy(
                src.at[2 * (rnd >> 2) + p, heads, rnd & 3, pl.ds(first + r, T // 2)],
                kv.at[slot, p, heads, pl.ds(r, T // 2)],
                sems.at[slot]).start(priority=p)
        return start

    def wo_pieces(u, p):
        def start(n):
            idx = (slice(None), p, _ds(u * DH + n * WR, WR))
            pltpu.make_async_copy(wo_hbm.at[idx], wo_v.at[idx], sems.at[u]).start(priority=p)
        return start

    def mlp_piece(p, c):
        src, dst = ((w3_hbm, w3_v), (w4_hbm, w4_v))[p]
        idx = (slice(None), _ds(c * WR, WR))
        pltpu.make_async_copy(src.at[idx], dst.at[idx], mlp_sem).start(priority=p)

    def alternate(starts):
        return lambda n: starts[n % 2](n // 2)

    lead, n_mlp = SKEW * G, FF // (2 * WR)
    lax.fori_loop(0, lead, lambda c, _: mlp_piece(1, c), None)
    x_copy = pltpu.make_async_copy(x_hbm, x_v, wq_sem)
    x_copy.start()

    def start_wq(c, _):
        for n in range(4):
            idx = (slice(None), n, _ds((c >> 2) * 8, 8), _ds((c & 3) * 1024, 1024))
            pltpu.make_async_copy(wq_hbm.at[idx], wq_v.at[idx], wq_sem).start(priority=n % 2)
    lax.fori_loop(0, 32, start_wq, None)

    def start_mlp(c, _):
        mlp_piece(0, c)
        mlp_piece(1, c + lead)
    lax.fori_loop(0, n_mlp - lead, start_mlp, None)

    def start_w3_k(t, _):
        start_k = kv_pieces(k_hbm, 0, t, 1, t)
        for n in range(G):
            mlp_piece(0, n_mlp - lead + t * G + n)
            start_k(n)
    lax.fori_loop(0, SKEW, start_w3_k, None)

    o_s[...] = jnp.zeros(o_s.shape, F32)
    x_copy.wait()
    _wait(wq_v, wq_sem)
    x = x_v[...].astype(F32)
    x = jnp.concatenate([x, x], axis=0)
    xn = _layernorm(x).astype(BF16)

    def q_step(issuing, u, _):
        if issuing:
            start = alternate([kv_pieces(k_hbm, 0, u + p * SKEW, p, u + p * SKEW) for p in range(2)])
        for a in range(4):
            h = 4 * u + a
            q_s[_ds(h * G, G), :] = _dot(xn, wq_v[:, :, :, _ds(h * DH, DH)].reshape(D, DH))
            if issuing:
                for n in range(4):
                    start(4 * a + n)
    lax.fori_loop(0, LAG[0], functools.partial(q_step, True), None)
    lax.fori_loop(LAG[0], NW, functools.partial(q_step, False), None)

    _wait(w3_v, mlp_sem)
    _wait(w4_v, mlp_sem)
    x1 = xn.astype(F32)
    hid = _dot(_layernorm(x1).astype(BF16), w3_v[...].reshape(FF, D), NT)
    hid = jax.nn.gelu(hid, approximate=True).astype(BF16)
    res_s[...] = x + x1 + _dot(hid, w4_v[...].reshape(FF, D))

    def head_row(rnd, p, i):
        return pl.ds((i * J + (rnd & 3)) * G + 2 * (rnd >> 2) + p, 1)

    def load_q(rnd, p):
        q = jnp.broadcast_to(q_s[head_row(rnd, p, 0), :], (G, DH))
        for i in range(1, G):
            q = jnp.where(row == i, q_s[head_row(rnd, p, i), :], q)
        return q.astype(BF16)

    def begin_unit(rnd, lo, last, t):
        slot = t & (RING - 1)
        _wait(kv.at[slot], sems.at[slot])
        starts = []
        for p in range(2):
            ahead, phase = t + LAG[p], (lo + LAG[p]) // NS
            if phase == 2 and last:
                starts.append(wo_pieces(ahead - 2 * NS, p))
            else:
                starts.append(kv_pieces((k_hbm, v_hbm)[phase % 2], rnd + phase // 2,
                                        ahead - phase * NS, p, ahead & (RING - 1)))
        return slot, alternate(starts)

    def per_head_dot(lhs, slot, p, dims, start):
        out = None
        for i in range(G):
            y = _dot(lhs, kv[slot, p, i], dims)
            out = y if out is None else jnp.where(row == i, y, out)
            start(p * G + i)
        return out

    def qk_step(rnd, lo, q, t, part_max):
        slot, start = begin_unit(rnd, lo, False, t)
        new = []
        for p in range(2):
            s = per_head_dot(q[p], slot, p, NT, start)
            s_s[t, p] = s
            new.append(jnp.maximum(part_max[p], s))
        return tuple(new)

    def pv_step(rnd, lo, last, row_max, t, carry):
        slot, start = begin_unit(rnd, lo, last, t)
        new = []
        for p in range(2):
            e = jnp.exp2((s_s[t - NS, p] - row_max[p]) * EXP2_SCALE)
            o = per_head_dot(e.astype(BF16), slot, p, NN, start)
            new.append((carry[p][0] + e, carry[p][1] + o))
        return tuple(new)

    spans = ((0, NS - LAG[1]), (NS - LAG[1], NS - LAG[0]), (NS - LAG[0], NS))

    def attention_round(rnd, _):
        q = (load_q(rnd, 0), load_q(rnd, 1))
        part_max = (jnp.full((G, T), -jnp.inf, F32),) * 2
        for lo, hi in spans:
            part_max = lax.fori_loop(lo, hi, functools.partial(qk_step, rnd, lo, q), part_max)
        row_max = tuple(jnp.broadcast_to(jnp.max(m, axis=-1, keepdims=True), (G, T)) for m in part_max)

        def pv_spans(which, last, carry):
            for lo, hi in which:
                step = functools.partial(pv_step, rnd, NS + lo, last, row_max)
                carry = lax.fori_loop(NS + lo, NS + hi, step, carry)
            return carry
        zero = jnp.zeros((G, T), F32)
        carry = pv_spans(spans[:1], False, ((zero, zero),) * 2)
        carry = lax.cond(rnd == NR - 1, functools.partial(pv_spans, spans[1:], True),
                         functools.partial(pv_spans, spans[1:], False), carry)
        for p in range(2):
            o = carry[p][1] / jnp.sum(carry[p][0], axis=-1, keepdims=True)
            for i in range(G):
                o_s[head_row(rnd, p, i), :] = o[i:i + 1, :]
    lax.fori_loop(0, NR, attention_round, None)

    def out_step(live, u, acc):
        rows = _ds(u * DH, DH)
        _wait(wo_v.at[:, :, rows], sems.at[u])
        for a in range(4):
            acc = acc + _dot(o_s[_ds((a * NW + u) * G, G), :].astype(BF16), wo_v[a // 2, a % 2, rows, :])
            for n in range(4 * a, 4 * a + 4):
                if n % 2 < live:
                    wo_pieces(u + LAG[n % 2], n % 2)(n // 2)
        return acc
    acc = res_s[...]
    for live, lo, hi in ((2, 0, NW - LAG[1]), (1, NW - LAG[1], NW - LAG[0]), (0, NW - LAG[0], NW)):
        acc = lax.fori_loop(lo, hi, functools.partial(out_step, live), acc)
    return acc[:B]


def _kernel(*refs):
    ins, out_hbm, scratch, (out_v, out_sem) = refs[:7], refs[7], refs[8:-2], refs[-2:]
    out_copy = pltpu.make_async_copy(out_v, out_hbm, out_sem)

    def scoped(*sems):
        out_v[...] = _compute(*ins, *scratch, *sems).astype(out_v.dtype)
        out_copy.start()
    pl.run_scoped(scoped, pltpu.SemaphoreType.DMA((RING,)),
                  pltpu.SemaphoreType.DMA(()), pltpu.SemaphoreType.DMA(()))
    out_copy.wait()


@jax.jit
def pallas_parallel_sum__sliding_block_cached__mixer_s_mlp__decode_kernel(
    A_x: jax.Array,
    A_k_cache: jax.Array,
    A_v_cache: jax.Array,
    A_wq: jax.Array,
    A_wo: jax.Array,
    B_x: jax.Array,
    B_w1: jax.Array,
    B_w2: jax.Array,
    B_w3: jax.Array,
    B_w4: jax.Array,
):
    assert A_x.shape == (B, 1, D) and A_k_cache.shape == A_v_cache.shape == (B, H, SK, DH)
    kv_shape = (B, G, J, SK, DH)
    wq_shape, wo_shape, mlp_shape = (2, 4, D // 8, H * DH), (2, 2, NW * DH, D), (2, FF // 2, D)
    hbm = pl.BlockSpec(memory_space=pltpu.HBM)
    out = pl.pallas_call(
        _kernel,
        out_shape=jax.ShapeDtypeStruct((B, D), A_x.dtype),
        in_specs=[hbm] * 7,
        out_specs=hbm,
        scratch_shapes=[
            pltpu.VMEM((RING, 2, G, T, DH), BF16),
            pltpu.VMEM((B, D), BF16),
            pltpu.VMEM(wq_shape, BF16),
            pltpu.VMEM(wo_shape, BF16),
            pltpu.VMEM(mlp_shape, BF16),
            pltpu.VMEM(mlp_shape, BF16),
            pltpu.VMEM((H * G, DH), F32),
            pltpu.VMEM((H * G, DH), F32),
            pltpu.VMEM((NS, 2, G, T), F32),
            pltpu.VMEM((G, D), F32),
            pltpu.VMEM((B, D), A_x.dtype),
            pltpu.SemaphoreType.DMA(()),
        ],
        compiler_params=pltpu.CompilerParams(vmem_limit_bytes=32 * 2**20),
    )(A_x.reshape(B, D), A_k_cache.reshape(kv_shape), A_v_cache.reshape(kv_shape),
      A_wq.reshape(wq_shape), A_wo.reshape(wo_shape),
      B_w3.T.reshape(mlp_shape),
      B_w4.reshape(mlp_shape))
    return out.reshape(B, 1, D)
```

```python
import functools
import math

import jax
import jax.numpy as jnp
from jax import lax
from jax.experimental import pallas as pl
from jax.experimental.pallas import tpu as pltpu

F32, BF16 = jnp.float32, jnp.bfloat16

B, H, SK, DH, D, FF = 4, 32, 8192, 128, 512, 1376
W = min(4096, max(256, SK // 4))
G = 8
J = H // G
T = 128
NS = W // T
NR = B * J // 2
RING = 8
SKEW = 3
LAG = (4, 4 + SKEW)
WR = 16
N_PROJ = 16
N_MLP = FF // (2 * WR)

NN = (((1,), (0,)), ((), ()))
NT = (((1,), (1,)), ((), ()))
EXP2_SCALE = DH ** -0.5 * math.log2(math.e)


def _layernorm(x, eps=1e-5):
    d = x - jnp.mean(x, axis=-1, keepdims=True)
    return d * lax.rsqrt(jnp.mean(d * d, axis=-1, keepdims=True) + eps)


def _dot(a, b, dims=NN):
    return lax.dot_general(a, b, dims, preferred_element_type=F32)


def _nothing(_):
    pass


def _per_head_dot(lhs, rhs, dims=NN, after=_nothing):
    out = None
    for i in range(G):
        y = _dot(lhs, rhs(i), dims)
        head = lax.broadcasted_iota(jnp.int32, y.shape, 0) & (G - 1)
        out = y if out is None else jnp.where(head == i, y, out)
        after(i)
    return out


def _ds(start, size):
    return pl.ds(pl.multiple_of(start, size), size)


def _wait(ref, sem):
    pltpu.make_async_copy(ref, ref, sem).wait()


def _body(x_hbm, k_hbm, v_hbm, wq_hbm, wo_hbm, w3_hbm, w4_hbm, out_hbm,
          kv, x_v, wq_v, wo_v, w3_v, w4_v, scores, out_v,
          sems, sem_a, sem_b):
    def kv_unit(src, rnd, s, p, slot):
        first = pl.multiple_of(SK - W + s * T, T)

        def start(n):
            heads, r = pl.ds(2 * (n % 4), 2), (n // 4) * (T // 2)
            pltpu.make_async_copy(
                src.at[2 * (rnd >> 2) + p, heads, rnd & 3, pl.ds(first + r, T // 2)],
                kv.at[slot, p, heads, pl.ds(r, T // 2)],
                sems.at[slot]).start(priority=p)
        return start

    def wq_unit(u):
        def start(n):
            c = 2 * u + n // 4
            idx = (slice(None), n % 4, _ds((c >> 2) * 8, 8), _ds((c & 3) * 1024, 1024))
            pltpu.make_async_copy(wq_hbm.at[idx], wq_v.at[idx], sem_a).start(priority=1)
        return start

    def wo_unit(u):
        def start(n):
            idx = (slice(None), n % 4, _ds((2 * u + n // 4) * WR, WR))
            pltpu.make_async_copy(wo_hbm.at[idx], wo_v.at[idx], sem_b).start(priority=0)
        return start

    def w3_piece(c, p):
        pltpu.make_async_copy(w3_hbm.at[:, _ds(c * WR, WR)], w3_v.at[c], sem_b).start(priority=p)

    def w4_piece(c, p, sem):
        pltpu.make_async_copy(w4_hbm.at[:, _ds(c * WR, WR)], w4_v.at[c], sem).start(priority=p)

    def w4_unit(u):
        return lambda n: w4_piece(u * G + n, 1, sems.at[u])

    def start_units(unit0, unit1):
        for n in range(G):
            unit0(n)
            unit1(n)

    lead = N_MLP - SKEW * G
    lax.fori_loop(0, lead, lambda c, _: w3_piece(c, 1), None)
    x_copy = pltpu.make_async_copy(x_hbm, x_v, sem_a)
    x_copy.start()
    lax.fori_loop(0, SKEW, lambda u, _: start_units(
        lambda n: w3_piece(lead + u * G + n, 0), wq_unit(u)), None)
    lax.fori_loop(0, N_PROJ - SKEW, lambda u, _: start_units(
        wo_unit(u), wq_unit(u + SKEW)), None)
    lax.fori_loop(0, SKEW, lambda u, _: start_units(
        wo_unit(N_PROJ - SKEW + u), kv_unit(k_hbm, 0, u, 1, u)), None)
    lax.fori_loop(0, LAG[0], lambda u, _: start_units(
        kv_unit(k_hbm, 0, u, 0, u), kv_unit(k_hbm, 0, u + SKEW, 1, u + SKEW)), None)
    x_copy.wait()
    _wait(wq_v, sem_a)
    _wait(wo_v, sem_b)
    _wait(w3_v, sem_b)

    x = x_v[...].astype(F32)
    xn = _layernorm(x).astype(BF16).astype(F32)
    hidden = _dot(_layernorm(xn).astype(BF16), w3_v[...].reshape(FF, D), NT)
    hidden = jax.nn.gelu(hidden, approximate=True).astype(BF16)

    def begin_unit(rnd, lo, last, t):
        slot = t & (RING - 1)
        _wait(kv.at[slot], sems.at[slot])
        units = []
        for p in range(2):
            ahead, phase = t + LAG[p], (lo + LAG[p]) // NS
            if phase < 2 or not last:
                units.append(kv_unit((k_hbm, v_hbm)[phase % 2], rnd + phase // 2,
                                     ahead - phase * NS, p, ahead & (RING - 1)))
            elif lo + LAG[0] < 2 * NS:
                units.append(w4_unit(ahead - 2 * NS))
            else:
                units.append(_nothing)
        return slot, lambda n: units[n % 2](n // 2)

    def key_step(rnd, lo, q, t, part_max):
        slot, start = begin_unit(rnd, lo, False, t)
        new = []
        for p in range(2):
            s = _per_head_dot(q[p], lambda i: kv[slot, p, i], NT, lambda i: start(p * G + i))
            scores[t, p] = s
            new.append(jnp.maximum(part_max[p], s))
        return tuple(new)

    def value_step(rnd, lo, last, row_max, t, sums):
        slot, start = begin_unit(rnd, lo, last, t)
        new = []
        for p in range(2):
            e = jnp.exp2((scores[t - NS, p] - row_max[p]) * EXP2_SCALE)
            o = _per_head_dot(e.astype(BF16), lambda i: kv[slot, p, i], NN, lambda i: start(p * G + i))
            new.append((sums[p][0] + e, sums[p][1] + o))
        return tuple(new)

    spans = ((0, NS - LAG[1]), (NS - LAG[1], NS - LAG[0]), (NS - LAG[0], NS))

    def attention_round(rnd, res):
        j = rnd & 3
        batch = lax.broadcasted_iota(jnp.int32, (B, D), 0)
        mine = [batch == 2 * (rnd >> 2) + p for p in range(2)]
        x_rows = [jnp.sum(jnp.where(m, xn, 0.0), axis=0, keepdims=True) for m in mine]
        q = _per_head_dot(
            jnp.concatenate([jnp.broadcast_to(r, (G, D)) for r in x_rows], axis=0).astype(BF16),
            lambda i: wq_v[:, :, :, _ds((i * J + j) * DH, DH)].reshape(D, DH))
        q = (q[:G].astype(BF16), q[G:].astype(BF16))

        part_max = (jnp.full((G, T), -jnp.inf, F32),) * 2
        for lo, hi in spans:
            part_max = lax.fori_loop(lo, hi, functools.partial(key_step, rnd, lo, q), part_max)
        row_max = tuple(jnp.broadcast_to(jnp.max(m, axis=-1, keepdims=True), (G, T)) for m in part_max)

        def value_span(span, last, sums):
            lo, hi = NS + span[0], NS + span[1]
            return lax.fori_loop(lo, hi, functools.partial(value_step, rnd, lo, last, row_max), sums)

        def finish(last, sums):
            sums = value_span(spans[1], last, sums)
            if last:
                lax.fori_loop(SKEW * G, N_MLP, lambda c, _: w4_piece(c, 0, sem_a), None)
            return value_span(spans[2], last, sums)

        zero = jnp.zeros((G, T), F32)
        sums = value_span(spans[0], False, ((zero, zero),) * 2)
        sums = lax.cond(rnd == NR - 1, functools.partial(finish, True),
                        functools.partial(finish, False), sums)

        o = jnp.concatenate([o / jnp.sum(e, axis=-1, keepdims=True) for e, o in sums], axis=0)
        y = _per_head_dot(o.astype(BF16), lambda i: wo_v[i // 4, i % 4, _ds(j * DH, DH), :])
        for p in range(2):
            res = jnp.where(mine[p], res + jnp.sum(y[p * G:(p + 1) * G], axis=0, keepdims=True), res)
        return res
    res = lax.fori_loop(0, NR, attention_round, x + xn)

    def w4_dot(lo, hi):
        return _dot(hidden[:, lo * 2 * WR:hi * 2 * WR], w4_v[lo:hi].reshape(-1, D))

    final = SKEW - 1
    _wait(w4_v.at[SKEW * G:], sem_a)
    for u in range(final):
        _wait(w4_v.at[u * G:(u + 1) * G], sems.at[u])
    res = res + w4_dot(SKEW * G, N_MLP) + w4_dot(0, final * G)
    _wait(w4_v.at[final * G:SKEW * G], sems.at[final])
    res = res + w4_dot(final * G, SKEW * G)

    out_v[...] = res.astype(out_v.dtype)
    out_copy = pltpu.make_async_copy(out_v, out_hbm, sem_b)
    out_copy.start()
    out_copy.wait()


def _kernel(*refs):
    dma = pltpu.SemaphoreType.DMA
    pl.run_scoped(functools.partial(_body, *refs), dma((RING,)), dma(()), dma(()))


@jax.jit
def pallas_parallel_sum__sliding_block_cached__mixer_s_mlp__decode_kernel(
    A_x: jax.Array,
    A_k_cache: jax.Array,
    A_v_cache: jax.Array,
    A_wq: jax.Array,
    A_wo: jax.Array,
    B_x: jax.Array,
    B_w1: jax.Array,
    B_w2: jax.Array,
    B_w3: jax.Array,
    B_w4: jax.Array,
):
    assert A_x.shape == (B, 1, D) and A_k_cache.shape == A_v_cache.shape == (B, H, SK, DH)
    kv_shape = (B, G, J, SK, DH)
    wq_shape, wo_shape, mlp_shape = (2, 4, D // 8, H * DH), (2, 4, J * DH, D), (2, FF // 2, D)
    hbm = pl.BlockSpec(memory_space=pltpu.HBM)
    out = pl.pallas_call(
        _kernel,
        out_shape=jax.ShapeDtypeStruct((B, D), A_x.dtype),
        in_specs=[hbm] * 7,
        out_specs=hbm,
        scratch_shapes=[
            pltpu.VMEM((RING, 2, G, T, DH), BF16),
            pltpu.VMEM((B, D), BF16),
            pltpu.VMEM(wq_shape, BF16),
            pltpu.VMEM(wo_shape, BF16),
            pltpu.VMEM((N_MLP, 2, WR, D), BF16),
            pltpu.VMEM((N_MLP, 2, WR, D), BF16),
            pltpu.VMEM((NS, 2, G, T), F32),
            pltpu.VMEM((B, D), A_x.dtype),
        ],
        compiler_params=pltpu.CompilerParams(vmem_limit_bytes=32 * 2**20),
    )(A_x.reshape(B, D), A_k_cache.reshape(kv_shape), A_v_cache.reshape(kv_shape),
      A_wq.reshape(wq_shape), A_wo.reshape(wo_shape),
      B_w3.T.reshape(mlp_shape),
      B_w4.reshape(mlp_shape))
    return out.reshape(B, 1, D)
```
